```python
import os as _os
_os.environ.setdefault("JAX_PLATFORMS", "cpu")
import jax
import jax.numpy as jnp

def _softmax(x, axis=-1):
    return jax.nn.softmax(x, axis=axis)
def _gelu(x):
    return jax.nn.gelu(x, approximate=True)
def _silu(x):
    return jax.nn.silu(x)
def _sigmoid(x):
    return jax.nn.sigmoid(x)
def _layernorm(x, axis=-1, eps=1e-5):
    m = jnp.mean(x, axis=axis, keepdims=True)
    v = jnp.var(x, axis=axis, keepdims=True)
    return (x - m) / jnp.sqrt(v + eps)
def _scatter_add(tgt, idx, src, axis=0):
    return tgt.at[idx].add(src)
def _segment_sum(src, seg, n):
    return jax.ops.segment_sum(src, seg, n)
class _Rng:
    def __init__(self, key):
        self._k = key
    def _next(self):
        self._k, sub = jax.random.split(self._k)
        return sub
    def normal(self, shape):
        return jax.random.normal(self._next(), shape, dtype=jnp.bfloat16)
    def randint(self, lo, hi, shape):
        return jax.random.randint(self._next(), shape, lo, hi, dtype=jnp.int32)
    def uniform(self, shape, lo=0.0, hi=1.0):
        return jax.random.uniform(self._next(), shape, jnp.bfloat16, lo, hi)
    def permutation(self, n):
        return jax.random.permutation(self._next(), n)


kernel_name = 'gated_mix__sliding_block_cached__dense_activation_silu__decode'

def setup_inputs():
    _rng = _Rng(jax.random.key(int.from_bytes(__import__("os").urandom(4), "little")))
    _w = (lambda a: (lambda t: t.astype(jnp.bfloat16) if jnp.issubdtype(t.dtype, jnp.floating) else t)(jnp.asarray(a)))
    def _A_setup():
        B, Sq, D = 2, 1, 1024
        Hq, Hkv, Sk, Dh = 32, 4, 32768, 128
        assert Hq % Hkv == 0, (Hq, Hkv)
        return {
            "x": _w((lambda *s: _rng.normal(s) * 0.05)(B, Sq, D)),
            "k_cache": _w((lambda *s: _rng.normal(s) * 3.2)(B, Hkv, Sk, Dh)),
            "v_cache": _w((lambda *s: _rng.normal(s) * 0.05)(B, Hkv, Sk, Dh)),
            "wq": _w((lambda *s: _rng.normal(s) * 3.2)(D, Hq * Dh) * (D ** -0.5)),
            "wo": _w((lambda *s: _rng.normal(s) * 0.05)(Hq * Dh, D) * ((Hq * Dh) ** -0.5)),
        }
    _A_in = _A_setup()

    def _B_setup():
        B, S, D, F = 2, 1, 1024, 3584
        return {
            "x": _w((lambda *s: _rng.normal(s) * 0.05)(B, S, D)),
            "w1": _w((lambda *s: _rng.normal(s) * 0.05)(D, F) * (D ** -0.5)),
            "w2": _w((lambda *s: _rng.normal(s) * 0.05)(F, D) * (F ** -0.5)),
        }
    _B_in = _B_setup()

    return {
        "A_x": _A_in["x"],
        "A_k_cache": _A_in["k_cache"],
        "A_v_cache": _A_in["v_cache"],
        "A_wq": _A_in["wq"],
        "A_wo": _A_in["wo"],
        "B_x": _B_in["x"],
        "B_w1": _B_in["w1"],
        "B_w2": _B_in["w2"],
        "gate_w": _w((lambda *s: _rng.normal(s) * 0.05)(1024) * 16.0),
    }

def reference(A_x, A_k_cache, A_v_cache, A_wq, A_wo, B_x, B_w1, B_w2, gate_w):
    def _A_ref(x, k_cache, v_cache, wq, wo):
        B, Sq, D = x.shape
        Hq, Dh = 32, 128
        Hkv, Sk = k_cache.shape[1], k_cache.shape[2]
        W = min(4096, max(256, Sk // 4))
        rep = Hq // Hkv
        q = (lambda x, *d: x.transpose(*d))((x @ wq).reshape(B, Sq, Hq, Dh), 0, 2, 1, 3)
        k = jnp.repeat(k_cache[:, :, Sk - W:, :], rep, axis=1)
        v = jnp.repeat(v_cache[:, :, Sk - W:, :], rep, axis=1)
        scores = jnp.einsum("bhqd,bhkd->bhqk", q, k) * (Dh ** -0.5)
        p = _softmax(scores, axis=-1)
        o = jnp.einsum("bhqk,bhkd->bhqd", p, v)
        return (lambda x, *d: x.transpose(*d))(o, 0, 2, 1, 3).reshape(B, Sq, Hq * Dh) @ wo

    def _B_ref(x, w1, w2):
        h = jnp.einsum("bsd,df->bsf", x, w1)
        h = _silu(h)
        out = jnp.einsum("bsf,fd->bsd", h, w2)
        return out

    x = A_x
    g = _sigmoid((x * gate_w).sum(-1, keepdims=True))
    a = _A_ref(x, A_k_cache, A_v_cache, A_wq, A_wo)
    b = _B_ref(x, B_w1, B_w2)
    return g * a + (1 - g) * b
```

```python
import functools

import jax
import jax.numpy as jnp
import jax.experimental.pallas as pl
import jax.experimental.pallas.tpu as pltpu

_HQ, _DH = 32, 128
_R = 8


def _build(B, D, Hkv, Sk, F, *, L=3, rq=128, ro=512, r1=128, r2=512, order="q1kvo2",
           dma_only=False):
    Hq, Dh, R = _HQ, _DH, _R
    rep = Hq // Hkv
    W = min(4096, max(256, Sk // 4))
    HD = Hq * Dh
    scale = Dh ** -0.5
    f32, bf16 = jnp.float32, jnp.bfloat16
    nq, no, n1, n2 = D // rq, HD // ro, D // r1, F // r2
    nkv = B * Hkv
    counts = {"q": nq, "k": nkv, "v": nkv, "o": no, "1": n1, "2": n2}
    base, tot = {}, 0
    for p in order:
        base[p] = tot
        tot += counts[p]

    def kernel(x_h, k_h, v_h, wq_h, wo_h, w1_h, w2_h, gw_h, out_ref,
               x_v, gw_v, wq_v, k_v, v_v, wo_v, w1_v, w2_v,
               xq_s, x1_s, qacc, q_s, p_s, l_s, o_s, hacc, h_s, acc_a, acc_b, sems, sem_s):

        def copy(p, j):
            sem = sems.at[base[p] + j]
            if p == "q":
                return pltpu.make_async_copy(wq_h.at[pl.ds(j * rq, rq), :], wq_v.at[j], sem)
            if p == "o":
                return pltpu.make_async_copy(wo_h.at[pl.ds(j * ro, ro), :], wo_v.at[j], sem)
            if p == "1":
                return pltpu.make_async_copy(w1_h.at[pl.ds(j * r1, r1), :], w1_v.at[j], sem)
            if p == "2":
                return pltpu.make_async_copy(w2_h.at[pl.ds(j * r2, r2), :], w2_v.at[j], sem)
            src, dst = (k_h, k_v) if p == "k" else (v_h, v_v)
            return pltpu.make_async_copy(
                src.at[j % B, j // B, pl.ds(Sk - W, W), :], dst.at[j], sem)

        def start_ahead(p, j):
            i = base[p] + j + L
            for p2 in order[order.index(p):]:
                lo, hi = base[p2], base[p2] + counts[p2]
                if isinstance(i, int):
                    if lo <= i < hi:
                        copy(p2, i - lo).start()
                    continue
                if hi <= base[p] + L or lo >= base[p] + counts[p] + L:
                    continue

                @pl.when(jnp.logical_and(i >= lo, i < hi))
                def _():
                    copy(p2, i - lo).start()

        cx = pltpu.make_async_copy(x_h, x_v, sem_s.at[0])
        cg = pltpu.make_async_copy(gw_h, gw_v, sem_s.at[1])
        first = order[0]
        copy(first, 0).start()
        cx.start()
        cg.start()
        for i in range(1, L):
            start_ahead(first, i - L)

        rows = jax.lax.broadcasted_iota(jnp.int32, (R, D), 0)
        rows128 = jax.lax.broadcasted_iota(jnp.int32, (R, 128), 0)
        cx.wait()
        x8 = jnp.zeros((R, D), f32)
        for b in range(B):
            x8 = jnp.where(rows == b, jnp.broadcast_to(x_v[b].astype(f32), (R, D)), x8)
        x8b = x8.astype(bf16)
        for j in range(nq):
            xq_s[j] = x8b[:, j * rq:(j + 1) * rq]
        for j in range(n1):
            x1_s[j] = x8b[:, j * r1:(j + 1) * r1]
        cg.wait()
        gw = gw_v[...].astype(f32).reshape(1, D)
        gate = jax.nn.sigmoid(jnp.sum(x8 * gw, axis=1, keepdims=True))

        def run(p, compute):
            def body(j, c):
                copy(p, j).wait()
                start_ahead(p, j)
                if not dma_only:
                    compute(j)
                return c
            jax.lax.fori_loop(0, counts[p], body, 0)

        def phase_q():
            qacc[...] = jnp.zeros_like(qacc)

            def comp(j):
                qacc[...] += jnp.dot(xq_s[j], wq_v[j], preferred_element_type=f32)
            run("q", comp)
            for g in range(Hkv):
                for b in range(B):
                    t = jnp.zeros((rep, Dh), f32)
                    for h in range(rep):
                        c0 = (g * rep + h) * Dh
                        t = jnp.where(rows128 == h,
                                      jnp.broadcast_to(qacc[b:b + 1, c0:c0 + Dh], (rep, Dh)), t)
                    q_s[g * B + b] = t.astype(bf16)

        def phase_k():
            def comp(j):
                s = jax.lax.dot_general(q_s[j], k_v[j], (((1,), (1,)), ((), ())),
                                        preferred_element_type=f32) * scale
                m = jnp.max(s, axis=1, keepdims=True)
                e = jnp.exp(s - m)
                l_s[j] = jnp.broadcast_to(jnp.sum(e, axis=1, keepdims=True), (rep, Dh))
                p_s[j] = e.astype(bf16)
            run("k", comp)

        def phase_v():
            def comp(j):
                o = jnp.dot(p_s[j], v_v[j], preferred_element_type=f32)
                l_s[j] = o / l_s[j]
            run("v", comp)
            hpc = ro // Dh
            for g in range(Hkv):
                for h in range(rep):
                    t = jnp.zeros((R, Dh), f32)
                    for b in range(B):
                        t = jnp.where(rows128 == b,
                                      jnp.broadcast_to(l_s[g * B + b, h:h + 1, :], (R, Dh)), t)
                    hh = g * rep + h
                    c0 = (hh % hpc) * Dh
                    o_s[hh // hpc, :, c0:c0 + Dh] = t.astype(bf16)

        def phase_o():
            acc_a[...] = jnp.zeros_like(acc_a)

            def comp(j):
                acc_a[...] += jnp.dot(o_s[j], wo_v[j], preferred_element_type=f32)
            run("o", comp)

        def phase_1():
            hacc[...] = jnp.zeros_like(hacc)

            def comp(j):
                hacc[...] += jnp.dot(x1_s[j], w1_v[j], preferred_element_type=f32)
            run("1", comp)
            for j in range(n2):
                hv = hacc[:, j * r2:(j + 1) * r2]
                h_s[j] = (hv * jax.nn.sigmoid(hv)).astype(bf16)

        def phase_2():
            acc_b[...] = jnp.zeros_like(acc_b)

            def comp(j):
                acc_b[...] += jnp.dot(h_s[j], w2_v[j], preferred_element_type=f32)
            run("2", comp)

        phases = {"q": phase_q, "k": phase_k, "v": phase_v, "o": phase_o,
                  "1": phase_1, "2": phase_2}
        for p in order:
            phases[p]()

        res = gate * acc_a[...] + (1.0 - gate) * acc_b[...]
        for b in range(B):
            out_ref[b] = res[b:b + 1, :].astype(out_ref.dtype)

    any_spec = pl.BlockSpec(memory_space=pl.ANY)
    return pl.pallas_call(
        kernel,
        out_shape=jax.ShapeDtypeStruct((B, 1, D), bf16),
        in_specs=[any_spec] * 8,
        out_specs=pl.BlockSpec(memory_space=pltpu.VMEM),
        scratch_shapes=[
            pltpu.VMEM((B, 1, D), bf16),
            pltpu.VMEM((D,), bf16),
            pltpu.VMEM((nq, rq, HD), bf16),
            pltpu.VMEM((nkv, W, Dh), bf16),
            pltpu.VMEM((nkv, W, Dh), bf16),
            pltpu.VMEM((no, ro, D), bf16),
            pltpu.VMEM((n1, r1, F), bf16),
            pltpu.VMEM((n2, r2, D), bf16),
            pltpu.VMEM((nq, R, rq), bf16),
            pltpu.VMEM((n1, R, r1), bf16),
            pltpu.VMEM((R, HD), f32),
            pltpu.VMEM((nkv, rep, Dh), bf16),
            pltpu.VMEM((nkv, rep, W), bf16),
            pltpu.VMEM((nkv, rep, Dh), f32),
            pltpu.VMEM((no, R, ro), bf16),
            pltpu.VMEM((R, F), f32),
            pltpu.VMEM((n2, R, r2), bf16),
            pltpu.VMEM((R, D), f32),
            pltpu.VMEM((R, D), f32),
            pltpu.SemaphoreType.DMA((tot,)),
            pltpu.SemaphoreType.DMA((2,)),
        ],
        compiler_params=pltpu.CompilerParams(vmem_limit_bytes=80 * 1024 * 1024),
    )


@jax.jit
def pallas_gated_mix__sliding_block_cached__dense_activation_silu__decode_kernel(
    A_x: jax.Array,
    A_k_cache: jax.Array,
    A_v_cache: jax.Array,
    A_wq: jax.Array,
    A_wo: jax.Array,
    B_x: jax.Array,
    B_w1: jax.Array,
    B_w2: jax.Array,
    gate_w: jax.Array,
):
    B, Sq, D = A_x.shape
    Hkv, Sk = A_k_cache.shape[1], A_k_cache.shape[2]
    F = B_w1.shape[1]
    call = _build(B, D, Hkv, Sk, F)
    return call(A_x, A_k_cache, A_v_cache, A_wq, A_wo, B_w1, B_w2, gate_w)
```

```python
import jax
import jax.numpy as jnp
import jax.experimental.pallas as pl
import jax.experimental.pallas.tpu as pltpu

_HQ, _DH = 32, 128
_R = 8


def _build(B, D, Hkv, Sk, F, *, L=3, rq=256, ro=1024, r1=256, mq=4, mo=2, m1=4, mk=4,
           w2c=(1024, 1024, 512, 384, 256, 128, 128, 128), order="q1kvo2"):
    Hq, Dh, R = _HQ, _DH, _R
    rep = Hq // Hkv
    W = min(4096, max(256, Sk // 4))
    HD = Hq * Dh
    scale = Dh ** -0.5
    f32, bf16 = jnp.float32, jnp.bfloat16
    nq, no, n1 = D // rq, HD // ro, D // r1
    nkv = B * Hkv
    assert sum(w2c) == F and Hkv % mk == 0
    w2o = [sum(w2c[:i]) for i in range(len(w2c))]
    mult = {"q": mq, "k": mk, "v": mk, "o": mo, "1": m1}
    counts = {"q": nq // mq, "k": nkv // mk, "v": nkv // mk, "o": no // mo, "1": n1 // m1,
              "2": len(w2c)}
    base, tot = {}, 0
    for p in order:
        base[p] = tot
        tot += counts[p]

    def kernel(x_h, k_h, v_h, wq_h, wo_h, w1_h, w2_h, gw_h, out_ref,
               x_v, gw_v, wq_v, k_v, v_v, wo_v, w1_v, w2_v,
               xq_s, x1_s, qacc, q_s, p_s, l_s, o_s, hacc, h_s, acc_a, sems, sem_s):

        def copy(p, j):
            sem = sems.at[base[p] + j]
            if p == "2":
                sl = pl.ds(w2o[j], w2c[j])
                return pltpu.make_async_copy(w2_h.at[sl, :], w2_v.at[sl, :], sem)
            if p in "qo1":
                src, dst, r = {"q": (wq_h, wq_v, rq), "o": (wo_h, wo_v, ro),
                               "1": (w1_h, w1_v, r1)}[p]
                sl = pl.ds(j * r * mult[p], r * mult[p])
                return pltpu.make_async_copy(src.at[sl, :], dst.at[sl, :], sem)
            src, dst = (k_h, k_v) if p == "k" else (v_h, v_v)
            b, g0 = (j * mk) // Hkv, (j * mk) % Hkv
            return pltpu.make_async_copy(
                src.at[b, pl.ds(g0, mk), pl.ds(Sk - W, W), :], dst.at[pl.ds(j * mk, mk)], sem)

        def start_ahead(p, j):
            i = base[p] + j + L
            for p2 in order:
                if base[p2] <= i < base[p2] + counts[p2]:
                    copy(p2, i - base[p2]).start()

        cx = pltpu.make_async_copy(x_h, x_v, sem_s.at[0])
        cg = pltpu.make_async_copy(gw_h, gw_v, sem_s.at[1])
        first = order[0]
        copy(first, 0).start()
        cx.start()
        cg.start()
        for i in range(1, L):
            start_ahead(first, i - L)

        rows = jax.lax.broadcasted_iota(jnp.int32, (R, D), 0)
        rows128 = jax.lax.broadcasted_iota(jnp.int32, (R, 128), 0)
        cx.wait()
        x8 = jnp.zeros((R, D), f32)
        xf = x_v[...].astype(f32)
        for b in range(B):
            x8 = jnp.where(rows == b, jnp.broadcast_to(xf[b:b + 1, :], (R, D)), x8)
        x8b = x8.astype(bf16)
        for j in range(nq):
            xq_s[j] = x8b[:, j * rq:(j + 1) * rq]
        for j in range(n1):
            x1_s[j] = x8b[:, j * r1:(j + 1) * r1]
        cg.wait()
        gw = gw_v[...].astype(f32).reshape(1, D)
        gate = jax.nn.sigmoid(jnp.sum(x8 * gw, axis=1, keepdims=True))

        def run(p, compute):
            for j in range(counts[p]):
                copy(p, j).wait()
                start_ahead(p, j)

                def body(t, c):
                    compute(j * mult[p] + t)
                    return c
                jax.lax.fori_loop(0, mult[p], body, 0)

        def rows_of(ref, j, r):
            return ref[pl.ds(pl.multiple_of(j * r, r), r), :]

        def phase_q():
            qacc[...] = jnp.zeros_like(qacc)

            def comp(j):
                qacc[...] += jnp.dot(xq_s[j], rows_of(wq_v, j, rq), preferred_element_type=f32)
            run("q", comp)
            for g in range(Hkv):
                for b in range(B):
                    t = jnp.zeros((rep, Dh), f32)
                    for h in range(rep):
                        c0 = (g * rep + h) * Dh
                        t = jnp.where(rows128 == h,
                                      jnp.broadcast_to(qacc[b:b + 1, c0:c0 + Dh], (rep, Dh)), t)
                    q_s[b * Hkv + g] = t.astype(bf16)

        def phase_k():
            def comp(j):
                s = jax.lax.dot_general(q_s[j], k_v[j], (((1,), (1,)), ((), ())),
                                        preferred_element_type=f32) * scale
                m = jnp.max(s, axis=1, keepdims=True)
                e = jnp.exp(s - m)
                l_s[j] = jnp.broadcast_to(jnp.sum(e, axis=1, keepdims=True), (rep, Dh))
                p_s[j] = e.astype(bf16)
            run("k", comp)

        def phase_v():
            def comp(j):
                o = jnp.dot(p_s[j], v_v[j], preferred_element_type=f32)
                l_s[j] = o / l_s[j]
            run("v", comp)
            hpc = ro // Dh
            for g in range(Hkv):
                for h in range(rep):
                    t = jnp.zeros((R, Dh), f32)
                    for b in range(B):
                        t = jnp.where(rows128 == b,
                                      jnp.broadcast_to(l_s[b * Hkv + g, h:h + 1, :], (R, Dh)), t)
                    hh = g * rep + h
                    c0 = (hh % hpc) * Dh
                    o_s[hh // hpc, :, c0:c0 + Dh] = t.astype(bf16)

        def phase_o():
            acc_a[...] = jnp.zeros_like(acc_a)

            def comp(j):
                acc_a[...] += jnp.dot(o_s[j], rows_of(wo_v, j, ro), preferred_element_type=f32)
            run("o", comp)

        def phase_1():
            hacc[...] = jnp.zeros_like(hacc)

            def comp(j):
                hacc[...] += jnp.dot(x1_s[j], rows_of(w1_v, j, r1), preferred_element_type=f32)
            run("1", comp)
            hv = hacc[...]
            h_s[...] = (hv * jax.nn.sigmoid(hv)).astype(bf16)

        def phase_2():
            acc = jnp.zeros((R, D), f32)
            ga = gate * acc_a[...]
            for j in range(len(w2c)):
                copy("2", j).wait()
                start_ahead("2", j)
                acc = acc + jnp.dot(h_s[:, w2o[j]:w2o[j] + w2c[j]],
                                    w2_v[w2o[j]:w2o[j] + w2c[j], :],
                                    preferred_element_type=f32)
            res = ga + (1.0 - gate) * acc
            out_ref[...] = res[:B, :].astype(out_ref.dtype)

        phases = {"q": phase_q, "k": phase_k, "v": phase_v, "o": phase_o,
                  "1": phase_1, "2": phase_2}
        for p in order:
            phases[p]()

    any_spec = pl.BlockSpec(memory_space=pl.ANY)
    return pl.pallas_call(
        kernel,
        out_shape=jax.ShapeDtypeStruct((B, D), bf16),
        in_specs=[any_spec] * 8,
        out_specs=pl.BlockSpec(memory_space=pltpu.VMEM),
        scratch_shapes=[
            pltpu.VMEM((B, D), bf16),
            pltpu.VMEM((D,), bf16),
            pltpu.VMEM((D, HD), bf16),
            pltpu.VMEM((nkv, W, Dh), bf16),
            pltpu.VMEM((nkv, W, Dh), bf16),
            pltpu.VMEM((HD, D), bf16),
            pltpu.VMEM((D, F), bf16),
            pltpu.VMEM((F, D), bf16),
            pltpu.VMEM((nq, R, rq), bf16),
            pltpu.VMEM((n1, R, r1), bf16),
            pltpu.VMEM((R, HD), f32),
            pltpu.VMEM((nkv, rep, Dh), bf16),
            pltpu.VMEM((nkv, rep, W), bf16),
            pltpu.VMEM((nkv, rep, Dh), f32),
            pltpu.VMEM((no, R, ro), bf16),
            pltpu.VMEM((R, F), f32),
            pltpu.VMEM((R, F), bf16),
            pltpu.VMEM((R, D), f32),
            pltpu.SemaphoreType.DMA((tot,)),
            pltpu.SemaphoreType.DMA((2,)),
        ],
        compiler_params=pltpu.CompilerParams(vmem_limit_bytes=80 * 1024 * 1024),
    )


@jax.jit
def pallas_gated_mix__sliding_block_cached__dense_activation_silu__decode_kernel(
    A_x: jax.Array,
    A_k_cache: jax.Array,
    A_v_cache: jax.Array,
    A_wq: jax.Array,
    A_wo: jax.Array,
    B_x: jax.Array,
    B_w1: jax.Array,
    B_w2: jax.Array,
    gate_w: jax.Array,
):
    B, Sq, D = A_x.shape
    Hkv, Sk = A_k_cache.shape[1], A_k_cache.shape[2]
    F = B_w1.shape[1]
    call = _build(B, D, Hkv, Sk, F)
    out = call(A_x.reshape(B * Sq, D), A_k_cache, A_v_cache, A_wq, A_wo, B_w1, B_w2, gate_w)
    return out.reshape(B, Sq, D)
```
